```python
import jax
import jax.numpy as jnp

def _softmax(x, axis=-1):
    return jax.nn.softmax(x, axis=axis)

def _gelu(x):
    return jax.nn.gelu(x, approximate=True)

def _silu(x):
    return jax.nn.silu(x)

def _sigmoid(x):
    return jax.nn.sigmoid(x)

def _layernorm(x, axis=-1, eps=1e-05):
    m = jnp.mean(x, axis=axis, keepdims=True)
    v = jnp.var(x, axis=axis, keepdims=True)
    return (x - m) / jnp.sqrt(v + eps)

def _scatter_add(tgt, idx, src, axis=0):
    return tgt.at[idx].add(src)

def _segment_sum(src, seg, n):
    return jax.ops.segment_sum(src, seg, n)

class _Rng:

    def __init__(self, key):
        self._k = key

    def _next(self):
        self._k, sub = jax.random.split(self._k)
        return sub

    def normal(self, shape):
        return jax.random.normal(self._next(), shape, dtype=jnp.bfloat16)

    def randint(self, lo, hi, shape):
        return jax.random.randint(self._next(), shape, lo, hi, dtype=jnp.int32)

    def uniform(self, shape, lo=0.0, hi=1.0):
        return jax.random.uniform(self._next(), shape, jnp.bfloat16, lo, hi)

    def permutation(self, n):
        return jax.random.permutation(self._next(), n)
kernel_name = 'adaLN_cond__sliding_block_cached__glu_gated_swiglu__decode'

def setup_inputs():
    _rng = _Rng(jax.random.key(int.from_bytes(__import__("os").urandom(4), "little")))
    _w = lambda a: (lambda t: t.astype(jnp.bfloat16) if jnp.issubdtype(t.dtype, jnp.floating) else t)(jnp.asarray(a))

    def _A_setup():
        B, Sq, D = (2, 1, 512)
        Hq, Hkv, Sk, Dh = (32, 32, 16384, 128)
        assert Hq % Hkv == 0, (Hq, Hkv)
        return {'x': _w((lambda *s: _rng.normal(s) * 0.05)(B, Sq, D)), 'k_cache': _w((lambda *s: _rng.normal(s) * 0.05)(B, Hkv, Sk, Dh)), 'v_cache': _w((lambda *s: _rng.normal(s) * 0.05)(B, Hkv, Sk, Dh)), 'wq': _w((lambda *s: _rng.normal(s) * 0.05)(D, Hq * Dh) * D ** (-0.5)), 'wo': _w((lambda *s: _rng.normal(s) * 0.05)(Hq * Dh, D) * (Hq * Dh) ** (-0.5))}
    _A_in = _A_setup()

    def _B_setup():
        B, S, D, F = (2, 1, 512, 1376)
        return {'x': _w((lambda *s: _rng.normal(s) * 0.05)(B, S, D)), 'w1': _w((lambda *s: _rng.normal(s) * 0.05)(D, F) * (2.0 / D) ** 0.5), 'w3': _w((lambda *s: _rng.normal(s) * 0.05)(D, F) * (2.0 / D) ** 0.5), 'w2': _w((lambda *s: _rng.normal(s) * 0.05)(F, D) * (2.0 / F) ** 0.5)}
    _B_in = _B_setup()
    return {'A_x': _A_in['x'], 'A_k_cache': _A_in['k_cache'], 'A_v_cache': _A_in['v_cache'], 'A_wq': _A_in['wq'], 'A_wo': _A_in['wo'], 'B_x': _B_in['x'], 'B_w1': _B_in['w1'], 'B_w3': _B_in['w3'], 'B_w2': _B_in['w2'], 'c': _w((lambda *s: _rng.normal(s) * 0.05)(2, 512)), 'w_mod': _w((lambda *s: _rng.normal(s) * 0.05)(512, 6 * 512) * 512 ** (-0.5))}

def reference(A_x, A_k_cache, A_v_cache, A_wq, A_wo, B_x, B_w1, B_w3, B_w2, c, w_mod):

    def _A_ref(x, k_cache, v_cache, wq, wo):
        B, Sq, D = x.shape
        Hq, Dh = (32, 128)
        Hkv, Sk = (k_cache.shape[1], k_cache.shape[2])
        W = min(4096, max(256, Sk // 4))
        rep = Hq // Hkv
        q = (lambda x, *d: x.transpose(*d))((x @ wq).reshape(B, Sq, Hq, Dh), 0, 2, 1, 3)
        k = jnp.repeat(k_cache[:, :, Sk - W:, :], rep, axis=1)
        v = jnp.repeat(v_cache[:, :, Sk - W:, :], rep, axis=1)
        scores = jnp.einsum('bhqd,bhkd->bhqk', q, k) * Dh ** (-0.5)
        p = _softmax(scores, axis=-1)
        o = jnp.einsum('bhqk,bhkd->bhqd', p, v)
        return (lambda x, *d: x.transpose(*d))(o, 0, 2, 1, 3).reshape(B, Sq, Hq * Dh) @ wo

    def _B_ref(x, w1, w3, w2):
        gate = jnp.einsum('bsd,df->bsf', x, w1)
        up = jnp.einsum('bsd,df->bsf', x, w3)
        h = _silu(gate) * up
        out = jnp.einsum('bsf,fd->bsd', h, w2)
        return out
    x = A_x
    mod = (_silu(c) @ w_mod).reshape(c.shape[0], 6, 1, -1)
    sa, ca, ga, sb, cb, gb = (mod[:, 0].copy(), mod[:, 1].copy(), mod[:, 2].copy(), mod[:, 3].copy(), mod[:, 4].copy(), mod[:, 5].copy())
    h = _layernorm(x, axis=-1) * (1 + ca) + sa
    x = x + ga * _A_ref(h, A_k_cache, A_v_cache, A_wq, A_wo)
    h = _layernorm(x, axis=-1) * (1 + cb) + sb
    x = x + gb * _B_ref(h, B_w1, B_w3, B_w2)
    return x
```

```python
import functools
import jax
import jax.numpy as jnp
from jax import lax
import jax.experimental.pallas as pl
import jax.experimental.pallas.tpu as pltpu

B, D, H, DH, SK, F = 2, 512, 32, 128, 16384, 1376
W = min(4096, max(256, SK // 4))
BF, F32 = jnp.bfloat16, jnp.float32


def _layernorm(x, eps=1e-5):
    m = jnp.mean(x, axis=-1, keepdims=True)
    d = x - m
    v = jnp.mean(d * d, axis=-1, keepdims=True)
    return d / jnp.sqrt(v + eps)


def _nt(a, b):
    return lax.dot_general(a, b, (((1,), (1,)), ((), ())), preferred_element_type=F32)


def _nn(a, b):
    return jnp.dot(a, b, preferred_element_type=F32)


def make(rows=128, nbuf=4, voff=256, wrows=16, wcols=1024, compute=True, MP=8):
    def kernel(x_hbm, k_hbm, v_hbm, wq_hbm, wo_hbm, w1_hbm, w3_hbm, w2_hbm, c_hbm, wm_hbm,
               o_ref,
               x_v, c_v, wm_v, wq_v, wo_v, w1_v, w3_v, w2_v, k_v, v_v, q_s, o_s,
               kv_sem, w_sem):
        def start_2d(src, dst, sem, pr=wrows, pc=wcols):
            R, C = src.shape
            pc = min(pc, C)
            i = 0
            for r in range(0, R, pr):
                for cc in range(0, C, pc):
                    pltpu.make_async_copy(src.at[pl.ds(r, pr), pl.ds(cc, pc)],
                                          dst.at[pl.ds(r, pr), pl.ds(cc, pc)], sem).start(priority=i % 2)
                    i += 1

        def wait_all(dst, sem):
            pltpu.make_async_copy(dst, dst, sem).wait()

        def start_kv(bh, s):
            for r in range(0, W, rows):
                rv = (r + voff) % W
                pltpu.make_async_copy(k_hbm.at[bh, pl.ds(SK - W + r, rows), :],
                                      k_v.at[s, pl.ds(r, rows)], kv_sem.at[0, s]).start(priority=0)
                pltpu.make_async_copy(v_hbm.at[bh, pl.ds(SK - W + rv, rows), :],
                                      v_v.at[s, pl.ds(rv, rows)], kv_sem.at[1, s]).start(priority=1)

        cx = pltpu.make_async_copy(x_hbm, x_v, w_sem.at[0]); cx.start()
        cc_ = pltpu.make_async_copy(c_hbm, c_v, w_sem.at[1]); cc_.start(priority=1)
        start_2d(wm_hbm, wm_v, w_sem.at[2])
        start_2d(wq_hbm, wq_v, w_sem.at[3])
        cx.wait(); cc_.wait()
        wait_all(wm_v, w_sem.at[2])
        c = c_v[...].astype(F32)
        sc = (c * jax.nn.sigmoid(c)).astype(BF)
        mod = _nn(sc, wm_v[...])
        sa, ca, ga, sb, cb, gb = [mod[:, i * D:(i + 1) * D] for i in range(6)]
        x = x_v[...].astype(F32)
        h = (_layernorm(x) * (1.0 + ca) + sa).astype(BF)
        start_kv(0, 0)
        wait_all(wq_v, w_sem.at[3])
        q = _nn(h, wq_v[...])
        for hh in range(H):
            q_s[hh] = q[:, hh * DH:(hh + 1) * DH]
        start_kv(H, 1)
        start_2d(wo_hbm, wo_v, w_sem.at[4], pr=wrows * 2)
        scale = DH ** -0.5

        def head(hh, b, s):
            wait_all(k_v.at[s], kv_sem.at[0, s])
            wait_all(v_v.at[s], kv_sem.at[1, s])
            if compute:
                qh = q_s[hh].astype(BF)
                sc_ = _nt(qh, k_v[s]) * scale
                m = jnp.max(sc_, axis=-1, keepdims=True)
                p = jnp.exp(sc_ - m)
                l = jnp.sum(p, axis=-1, keepdims=True)
                o = _nn(p.astype(BF), v_v[s]) / l
                return o
            return jnp.zeros((2, DH), F32)

        row = lax.broadcasted_iota(jnp.int32, (2, DH), 0)

        def pair(hh, acc, last):
            s0 = lax.bitwise_and(2 * hh, nbuf - 1)
            if not last:
                start_kv(hh + 1, lax.bitwise_and(2 * hh + 2, nbuf - 1))
            else:
                start_2d(w1_hbm, w1_v, w_sem.at[5], pr=32, pc=512)
            o0 = head(hh, 0, s0)
            if not last:
                start_kv(H + hh + 1, lax.bitwise_and(2 * hh + 3, nbuf - 1))
            else:
                start_2d(w3_hbm, w3_v, w_sem.at[6], pr=32, pc=512)
            o1 = head(hh, 1, s0 + 1)
            o = jnp.where(row == 0, o0, o1).astype(BF)
            return acc + _nn(o, wo_v[pl.ds(pl.multiple_of(hh * DH, DH), DH), :])

        wait_all(wo_v, w_sem.at[4])
        acc = lax.fori_loop(0, H - 1, lambda hh, a: pair(hh, a, False), jnp.zeros((2, D), F32))
        acc = pair(H - 1, acc, True)
        start_2d(w2_hbm, w2_v, w_sem.at[7], pr=32, pc=512)
        x1 = x + ga * acc
        h2 = (_layernorm(x1) * (1.0 + cb) + sb).astype(BF)
        wait_all(w1_v, w_sem.at[5])
        g = _nt(h2, w1_v[...])
        wait_all(w3_v, w_sem.at[6])
        u = _nt(h2, w3_v[...])
        a = (g * jax.nn.sigmoid(g) * u).astype(BF)
        wait_all(w2_v, w_sem.at[7])
        y = _nn(a, w2_v[...])
        o_ref[...] = (x1 + gb * y).astype(o_ref.dtype)

    def f(A_x, A_k_cache, A_v_cache, A_wq, A_wo, B_x, B_w1, B_w3, B_w2, c, w_mod):
        a = [A_x.reshape(B, D), A_k_cache.reshape(B * H, SK, DH), A_v_cache.reshape(B * H, SK, DH),
             A_wq, A_wo, B_w1.T, B_w3.T, B_w2, c, w_mod]
        V = pltpu.VMEM
        out = pl.pallas_call(
            kernel, out_shape=jax.ShapeDtypeStruct((B, D), BF),
            in_specs=[pl.BlockSpec(memory_space=pltpu.HBM)] * len(a),
            scratch_shapes=[V((B, D), BF), V((B, D), BF), V((D, 6 * D), BF), V((D, H * DH), BF), V((H * DH, D), BF),
                            V((F, D), BF), V((F, D), BF), V((F, D), BF),
                            V((nbuf, W, DH), BF), V((nbuf, W, DH), BF), V((H, B, DH), F32), V((H, B, DH), F32),
                            pltpu.SemaphoreType.DMA((2, nbuf)), pltpu.SemaphoreType.DMA((8,))],
            compiler_params=pltpu.CompilerParams(vmem_limit_bytes=100 * 2**20, disable_bounds_checks=True),
        )(*a)
        return out.reshape(B, 1, D)
    return f


_impl = make()


@jax.jit
def pallas_adaLN_cond__sliding_block_cached__glu_gated_swiglu__decode_kernel(
    A_x, A_k_cache, A_v_cache, A_wq, A_wo, B_x, B_w1, B_w3, B_w2, c, w_mod,
):
    return _impl(A_x, A_k_cache, A_v_cache, A_wq, A_wo, B_x, B_w1, B_w3, B_w2, c, w_mod)
```

```python
import jax
import jax.numpy as jnp
from jax import lax
import jax.experimental.pallas as pl
import jax.experimental.pallas.tpu as pltpu

B, D, H, DH, SK, F = 2, 512, 32, 128, 16384, 1376
W = min(4096, max(256, SK // 4))
BF, F32 = jnp.bfloat16, jnp.float32


def _layernorm(x, eps=1e-5):
    m = jnp.mean(x, axis=-1, keepdims=True)
    d = x - m
    v = jnp.mean(d * d, axis=-1, keepdims=True)
    return d / jnp.sqrt(v + eps)


def _nt(a, b):
    return lax.dot_general(a, b, (((1,), (1,)), ((), ())), preferred_element_type=F32)


def _nn(a, b):
    return jnp.dot(a, b, preferred_element_type=F32)


SEGS=((7,"w1",0,"w1",36),(23,"w1",7,"w3",20),(6,"w1",30,"w2",8),(20,"w3",0,"w2",14),(8,"w2",0,"w2",34),(1,None,0,"w2",42))
def make(rows=128, nbuf=4, voff=0, compute=True, wrot=0, wm_cols=1024, nobc=True, skip=(), groups=((0,1,2,3,4),(5,6,7,8),(9,10)),segs=SEGS,nseg1=2,early=True, kvloop=4):
    def kernel(x_hbm, k_hbm, v_hbm, wq_hbm, wo_hbm, w1_hbm, w3_hbm, w2_hbm, c_hbm, wm_hbm,
               o_ref,
               x_v, c_v, wm_v, wq_v, wo_v, w1_v, w3_v, w2_v, k_v, v_v, q_s,
               kv_sem, w_sem, w2_sem):
        def cp(src, dst, sem, r, pr, cc, pc):
            if not isinstance(r, int):
                r = pl.multiple_of(r, pr)
            return pltpu.make_async_copy(src.at[pl.ds(r, pr), pl.ds(cc, pc)],
                                         dst.at[pl.ds(r, pr), pl.ds(cc, pc)], sem)

        def start_w(name, src, dst, sem, pr, pc, per=1):
            if name in skip:
                return
            R, C = src.shape
            n = R // pr
            na = (n + 1) // 2
            nb = n - na
            semf = sem if callable(sem) else (lambda r: sem)

            def body(i, _):
                for u in range(per):
                    ra = (i * per + u) * pr
                    rb = ra + na * pr
                    for cc in range(0, C, pc):
                        cp(src, dst, semf(ra), ra, pr, cc, pc).start(priority=0)
                        cp(src, dst, semf(rb), rb, pr, cc, pc).start(priority=1)
            assert nb % per == 0
            lax.fori_loop(0, nb // per, body, None)
            if na > nb:
                for cc in range(0, C, pc):
                    cp(src, dst, semf(nb * pr), nb * pr, pr, cc, pc).start(priority=0)

        def wait_all(name, dst, sem):
            if name in skip:
                return
            pltpu.make_async_copy(dst, dst, sem).wait()

        def start_kv(bh, s):
            def body(i, _):
                for u in range(kvloop):
                    r = (i * kvloop + u) * rows
                    rv = lax.bitwise_and(r + voff, W - 1)
                    r = pl.multiple_of(r, rows)
                    rv = pl.multiple_of(rv, rows)
                    pltpu.make_async_copy(k_hbm.at[bh, pl.ds(SK - W + r, rows), :],
                                          k_v.at[s, pl.ds(r, rows)], kv_sem.at[0, s]).start(priority=0)
                    pltpu.make_async_copy(v_hbm.at[bh, pl.ds(SK - W + rv, rows), :],
                                          v_v.at[s, pl.ds(rv, rows)], kv_sem.at[1, s]).start(priority=1)
            lax.fori_loop(0, W // rows // kvloop, body, None)

        cx = pltpu.make_async_copy(x_hbm, x_v, w_sem.at[0]); cx.start()
        cc_ = pltpu.make_async_copy(c_hbm, c_v, w_sem.at[1]); cc_.start(priority=1)
        start_w("wm", wm_hbm, wm_v, w_sem.at[2], 8, wm_cols)
        start_w("wq", wq_hbm, wq_v, w_sem.at[3], 8, 2048, per=2)
        cx.wait(); cc_.wait()
        wait_all("wm", wm_v, w_sem.at[2])
        x = x_v[...].astype(F32)
        if compute:
            c = c_v[...].astype(F32)
            sc = (c * jax.nn.sigmoid(c)).astype(BF)
            mod = _nn(sc, wm_v[...])
            sa, ca, ga, sb, cb, gb = [mod[:, i * D:(i + 1) * D] for i in range(6)]
            h = (_layernorm(x) * (1.0 + ca) + sa).astype(BF)
        start_kv(0, 0)
        if early: start_kv(H, 1)
        wait_all("wq", wq_v, w_sem.at[3])
        if compute:
            q = _nn(h, wq_v[...])
            for hh in range(H):
                q_s[hh] = q[:, hh * DH:(hh + 1) * DH]
        if not early: start_kv(H, 1)
        start_w("wo", wo_hbm, wo_v, w_sem.at[4], 32, 512, per=4)
        scale = DH ** -0.5

        def head(hh, b, s):
            wait_all("k", k_v.at[s], kv_sem.at[0, s])
            wait_all("v", v_v.at[s], kv_sem.at[1, s])
            if compute:
                qh = q_s[hh].astype(BF)
                sc_ = _nt(qh, k_v[s]) * scale
                m = jnp.max(sc_, axis=-1, keepdims=True)
                p = jnp.exp(sc_ - m)
                l = jnp.sum(p, axis=-1, keepdims=True)
                o = _nn(p.astype(BF), v_v[s]) / l
                return o
            return jnp.zeros((2, DH), F32)

        def wchunk(name, ci):
            src, dst = {"w1": (w1_hbm, w1_v), "w3": (w3_hbm, w3_v), "w2": (w2_hbm, w2_v)}[name]
            if name == "w2":
                sem = w2_sem.at[ci // 4 if isinstance(ci, int) else lax.shift_right_logical(ci, 2)]
            else:
                sem = w_sem.at[5 if name == "w1" else 6]
            return cp(src, dst, sem, ci * 32, 32, 0, D)

        def tail_seg(n, n0, c0, n1, c1):
            if n == 1:
                if n0: wchunk(n0, c0).start(priority=0)
                if n1: wchunk(n1, c1).start(priority=1)
                return
            def body(i, _):
                if n0: wchunk(n0, c0 + i).start(priority=0)
                if n1: wchunk(n1, c1 + i).start(priority=1)
            lax.fori_loop(0, n, body, None)

        row = lax.broadcasted_iota(jnp.int32, (2, DH), 0)

        def pair(hh, acc, last):
            s0 = lax.bitwise_and(2 * hh, nbuf - 1)
            if not last:
                start_kv(hh + 1, lax.bitwise_and(2 * hh + 2, nbuf - 1))
            else:
                for sg in segs[:nseg1]: tail_seg(*sg)
            o0 = head(hh, 0, s0)
            if not last:
                start_kv(H + hh + 1, lax.bitwise_and(2 * hh + 3, nbuf - 1))
            else:
                for sg in segs[nseg1:]: tail_seg(*sg)
            o1 = head(hh, 1, s0 + 1)
            if not last:
                @pl.when(hh == 0)
                def _():
                    wait_all("wo", wo_v, w_sem.at[4])
            if not compute:
                return acc
            o = jnp.where(row == 0, o0, o1).astype(BF)
            return acc + _nn(o, wo_v[pl.ds(pl.multiple_of(hh * DH, DH), DH), :])

        acc = lax.fori_loop(0, H - 1, lambda hh, a: pair(hh, a, False), jnp.zeros((2, D), F32))
        acc = pair(H - 1, acc, True)
        wait_all("w1", w1_v, w_sem.at[5])
        if compute:
            x1 = x + ga * acc
            h2 = (_layernorm(x1) * (1.0 + cb) + sb).astype(BF)
            g = _nt(h2, w1_v[...])
        wait_all("w3", w3_v, w_sem.at[6])
        if compute:
            u = _nt(h2, w3_v[...])
            a = (g * jax.nn.sigmoid(g) * u).astype(BF)
        y = jnp.zeros((2, D), F32)
        for grp in groups:
            for i in grp:
                n = min(128, F - i * 128)
                wait_all("w2", w2_v.at[pl.ds(i * 128, n)], w2_sem.at[i])
            if compute:
                for i in grp:
                    r0 = i * 128
                    n = min(128, F - r0)
                    y = y + _nn(a[:, r0:r0 + n], w2_v[pl.ds(r0, n), :])
        if compute:
            o_ref[...] = (x1 + gb * y).astype(o_ref.dtype)
        else:
            o_ref[...] = x.astype(o_ref.dtype)

    def f(A_x, A_k_cache, A_v_cache, A_wq, A_wo, B_x, B_w1, B_w3, B_w2, c, w_mod):
        a = [A_x.reshape(B, D), A_k_cache.reshape(B * H, SK, DH), A_v_cache.reshape(B * H, SK, DH),
             A_wq, A_wo, B_w1.T, B_w3.T, B_w2, c, w_mod]
        V = pltpu.VMEM
        out = pl.pallas_call(
            kernel, out_shape=jax.ShapeDtypeStruct((B, D), BF),
            in_specs=[pl.BlockSpec(memory_space=pltpu.HBM)] * len(a),
            scratch_shapes=[V((B, D), BF), V((B, D), BF), V((D, 6 * D), BF), V((D, H * DH), BF), V((H * DH, D), BF),
                            V((F, D), BF), V((F, D), BF), V((F, D), BF),
                            V((nbuf, W, DH), BF), V((nbuf, W, DH), BF), V((H, B, DH), F32),
                            pltpu.SemaphoreType.DMA((2, nbuf)), pltpu.SemaphoreType.DMA((8,)),
                            pltpu.SemaphoreType.DMA((11,))],
            compiler_params=pltpu.CompilerParams(vmem_limit_bytes=100 * 2**20, disable_bounds_checks=nobc),
        )(*a)
        return out.reshape(B, 1, D)
    return f


_impl = make()


@jax.jit
def pallas_adaLN_cond__sliding_block_cached__glu_gated_swiglu__decode_kernel(
    A_x, A_k_cache, A_v_cache, A_wq, A_wo, B_x, B_w1, B_w3, B_w2, c, w_mod,
):
    return _impl(A_x, A_k_cache, A_v_cache, A_wq, A_wo, B_x, B_w1, B_w3, B_w2, c, w_mod)
```

```python
import jax
import jax.numpy as jnp
from jax import lax
import jax.experimental.pallas as pl
import jax.experimental.pallas.tpu as pltpu

B, D, H, DH, SK, F = 2, 512, 32, 128, 16384, 1376
W = min(4096, max(256, SK // 4))
BF, F32 = jnp.bfloat16, jnp.float32


def _layernorm(x, eps=1e-5):
    m = jnp.mean(x, axis=-1, keepdims=True)
    d = x - m
    v = jnp.mean(d * d, axis=-1, keepdims=True)
    return d / jnp.sqrt(v + eps)


def _nt(a, b):
    return lax.dot_general(a, b, (((1,), (1,)), ((), ())), preferred_element_type=F32)


def _nn(a, b):
    return jnp.dot(a, b, preferred_element_type=F32)


SEGS = ((21, "w1", 0, "w1", 22), (1, "w1", 21, "w3", 33), (9, "w3", 0, "w3", 34), (24, "w3", 9, "w2", 9),
        (9, "w2", 0, "w2", 33), (1, None, 0, "w2", 42))


def make(rows=128, compute=True, nobc=False, segs=SEGS, nseg1=4, groups=((0, 1, 2, 3), (4, 5, 6), (7, 8), (9, 10)), scopes=False):
    def kernel(x_hbm, k_hbm, v_hbm, wq_hbm, wo_hbm, w1_hbm, w3_hbm, w2_hbm, c_hbm, wm_hbm,
               o_ref,
               x_v, c_v, wm_v, wq_v, wo_v, w1_v, w3_v, w2_v, k_v, v_v, q_s,
               kv_sem, w_sem, w2_sem):
        def cp(src, dst, sem, r, pr, cc, pc):
            if not isinstance(r, int):
                r = pl.multiple_of(r, pr)
            return pltpu.make_async_copy(src.at[pl.ds(r, pr), pl.ds(cc, pc)],
                                         dst.at[pl.ds(r, pr), pl.ds(cc, pc)], sem)

        def wait_all(name, dst, sem):
            if scopes:
                with jax.named_scope("wait_" + name):
                    pltpu.make_async_copy(dst, dst, sem).wait()
            else:
                pltpu.make_async_copy(dst, dst, sem).wait()

        def start_kv(hh, s):
            def body(i, _):
                for b in range(B):
                    for half in range(2):
                        r = pl.multiple_of(i * rows, rows) + half * (W // 2)
                        pltpu.make_async_copy(k_hbm.at[hh + b * H, pl.ds(SK - W + r, rows), :],
                                              k_v.at[s, b, pl.ds(r, rows)], kv_sem.at[0, s]).start(priority=0)
                        pltpu.make_async_copy(v_hbm.at[hh + b * H, pl.ds(SK - W + r, rows), :],
                                              v_v.at[s, b, pl.ds(r, rows)], kv_sem.at[1, s]).start(priority=1)
            lax.fori_loop(0, W // 2 // rows, body, None)

        cx = pltpu.make_async_copy(x_hbm, x_v, w_sem.at[0]); cx.start()
        cc_ = pltpu.make_async_copy(c_hbm, c_v, w_sem.at[1]); cc_.start(priority=1)

        def p1(i, _):
            for half in range(2):
                for qd in range(4):
                    r = i * 8 + qd * 128
                    cp(wm_hbm, wm_v, w_sem.at[2], r, 8, half * 1536, 1536).start(priority=0)
                    cp(wq_hbm, wq_v, w_sem.at[3], r, 8, half * 2048, 2048).start(priority=1)
        lax.fori_loop(0, 16, p1, None)
        start_kv(0, 0)
        cx.wait(); cc_.wait()
        wait_all("wm", wm_v, w_sem.at[2])
        wait_all("wq", wq_v, w_sem.at[3])
        x = x_v[...].astype(F32)
        if compute:
            c = c_v[...].astype(F32)
            sc = (c * jax.nn.sigmoid(c)).astype(BF)
            mod = _nn(sc, wm_v[...])
            sa, ca, ga, sb, cb, gb = [mod[:, i * D:(i + 1) * D] for i in range(6)]
            h = (_layernorm(x) * (1.0 + ca) + sa).astype(BF)
            q = _nn(h, wq_v[...])
            for hh in range(H):
                q_s[hh] = q[:, hh * DH:(hh + 1) * DH]

        def p2(i, _):
            for st in range(8):
                cp(wo_hbm, wo_v, w_sem.at[4], i * 32 + st * 512, 32, 0, D).start(priority=st % 2)
        lax.fori_loop(0, 16, p2, None)
        scale = DH ** -0.5

        def head(hh, b, s):
            qh = q_s[hh].astype(BF)
            sc_ = _nt(qh, k_v[s, b]) * scale
            m = jnp.max(sc_, axis=-1, keepdims=True)
            p = jnp.exp(sc_ - m)
            l = jnp.sum(p, axis=-1, keepdims=True)
            return _nn(p.astype(BF), v_v[s, b]) / l

        def wchunk(name, ci):
            src, dst = {"w1": (w1_hbm, w1_v), "w3": (w3_hbm, w3_v), "w2": (w2_hbm, w2_v)}[name]
            if name == "w2":
                sem = w2_sem.at[ci // 4 if isinstance(ci, int) else lax.shift_right_logical(ci, 2)]
            else:
                sem = w_sem.at[5 if name == "w1" else 6]
            return cp(src, dst, sem, ci * 32, 32, 0, D)

        def tail_seg(n, n0, c0, n1, c1):
            if n == 1:
                if n0: wchunk(n0, c0).start(priority=0)
                if n1: wchunk(n1, c1).start(priority=1)
                return
            def body(i, _):
                if n0: wchunk(n0, c0 + i).start(priority=0)
                if n1: wchunk(n1, c1 + i).start(priority=1)
            lax.fori_loop(0, n, body, None)

        row = lax.broadcasted_iota(jnp.int32, (2, DH), 0)

        def pair(hh, acc, last):
            s = lax.bitwise_and(hh, 1)
            if not last:
                start_kv(hh + 1, 1 - s)
                @pl.when(hh == 0)
                def _():
                    wait_all("wo", wo_v, w_sem.at[4])
            else:
                for sg in segs[:nseg1]: tail_seg(*sg)
            wait_all("k", k_v.at[s], kv_sem.at[0, s])
            wait_all("v", v_v.at[s], kv_sem.at[1, s])
            if not compute:
                return acc
            o0 = head(hh, 0, s)
            o1 = head(hh, 1, s)
            o = jnp.where(row == 0, o0, o1).astype(BF)
            return acc + _nn(o, wo_v[pl.ds(pl.multiple_of(hh * DH, DH), DH), :])

        acc = lax.fori_loop(0, H - 1, lambda hh, a: pair(hh, a, False), jnp.zeros((2, D), F32))
        acc = pair(H - 1, acc, True)
        for sg in segs[nseg1:]: tail_seg(*sg)
        wait_all("w1", w1_v, w_sem.at[5])
        if compute:
            x1 = x + ga * acc
            h2 = (_layernorm(x1) * (1.0 + cb) + sb).astype(BF)
            g = _nt(h2, w1_v[...])
        wait_all("w3", w3_v, w_sem.at[6])
        if compute:
            u = _nt(h2, w3_v[...])
            a = (g * jax.nn.sigmoid(g) * u).astype(BF)
        y = jnp.zeros((2, D), F32)
        for grp in groups:
            for i in grp:
                n = min(128, F - i * 128)
                wait_all("w2_%d" % i, w2_v.at[pl.ds(i * 128, n)], w2_sem.at[i])
            if compute:
                for i in grp:
                    r0 = i * 128
                    n = min(128, F - r0)
                    y = y + _nn(a[:, r0:r0 + n], w2_v[pl.ds(r0, n), :])
        if compute:
            o_ref[...] = (x1 + gb * y).astype(o_ref.dtype)
        else:
            o_ref[...] = x.astype(o_ref.dtype)

    def f(A_x, A_k_cache, A_v_cache, A_wq, A_wo, B_x, B_w1, B_w3, B_w2, c, w_mod):
        a = [A_x.reshape(B, D), A_k_cache.reshape(B * H, SK, DH), A_v_cache.reshape(B * H, SK, DH),
             A_wq, A_wo, B_w1.T, B_w3.T, B_w2, c, w_mod]
        V = pltpu.VMEM
        out = pl.pallas_call(
            kernel, out_shape=jax.ShapeDtypeStruct((B, D), BF),
            in_specs=[pl.BlockSpec(memory_space=pltpu.HBM)] * len(a),
            scratch_shapes=[V((B, D), BF), V((B, D), BF), V((D, 6 * D), BF), V((D, H * DH), BF), V((H * DH, D), BF),
                            V((F, D), BF), V((F, D), BF), V((F, D), BF),
                            V((2, B, W, DH), BF), V((2, B, W, DH), BF), V((H, B, DH), F32),
                            pltpu.SemaphoreType.DMA((2, 2)), pltpu.SemaphoreType.DMA((8,)),
                            pltpu.SemaphoreType.DMA((11,))],
            compiler_params=pltpu.CompilerParams(vmem_limit_bytes=100 * 2**20, disable_bounds_checks=nobc),
        )(*a)
        return out.reshape(B, 1, D)
    return f


_impl = make()


@jax.jit
def pallas_adaLN_cond__sliding_block_cached__glu_gated_swiglu__decode_kernel(
    A_x, A_k_cache, A_v_cache, A_wq, A_wo, B_x, B_w1, B_w3, B_w2, c, w_mod,
):
    return _impl(A_x, A_k_cache, A_v_cache, A_wq, A_wo, B_x, B_w1, B_w3, B_w2, c, w_mod)
```

```python
import jax
import jax.numpy as jnp
from jax import lax
import jax.experimental.pallas as pl
import jax.experimental.pallas.tpu as pltpu

B, D, H, DH, SK, F = 2, 512, 32, 128, 16384, 1376
W = min(4096, max(256, SK // 4))
BF, F32 = jnp.bfloat16, jnp.float32


def _layernorm(x, eps=1e-5):
    m = jnp.mean(x, axis=-1, keepdims=True)
    d = x - m
    v = jnp.mean(d * d, axis=-1, keepdims=True)
    return d / jnp.sqrt(v + eps)


def _nt(a, b):
    return lax.dot_general(a, b, (((1,), (1,)), ((), ())), preferred_element_type=F32)


def _nn(a, b):
    return jnp.dot(a, b, preferred_element_type=F32)


SEGS = ((21, "w1", 0, "w1", 22), (1, "w1", 21, "w3", 33), (9, "w3", 0, "w3", 34), (24, "w3", 9, "w2", 9),
        (9, "w2", 0, "w2", 33), (1, None, 0, "w2", 42))


def kv_schedule(dk, dv, lag, rows=128):
    def stream(w, g, d):
        out = []
        for c in range(W // rows):
            r = (c * rows - d) % W
            out.append((w, g, ((r, rows),) if r + rows <= W else ((r, W - r), (0, r + rows - W))))
        return out
    rr = lambda ss: [s[i] for i in range(len(ss[0])) for s in ss]
    if lag is None:
        q0 = rr([stream(0, g, dk) for g in range(4)])
        q1 = rr([stream(1, g, dv) for g in range(4)])
    else:
        st = [stream(w, g, (dk, dv)[w]) for g in range(4) for w in (0, 1)]
        q0 = rr([s[0::2] for s in st])
        q1 = rr([s[1::2] for s in st])
        q1 = q1[lag:] + q1[:lag]
    return list(zip(q0, q1))


def make(dk=0, dv=64, lag=None, rows=128, compute=True, nobc=False, segs=SEGS, nseg1=1, groups=((0, 1, 2, 3), (4, 5, 6), (7, 8), (9, 10)), scopes=False):
    def kernel(x_hbm, k_hbm, v_hbm, wq_hbm, wo_hbm, w1_hbm, w3_hbm, w2_hbm, c_hbm, wm_hbm,
               o_ref,
               x_v, c_v, wm_v, wq_v, wo_v, w1_v, w3_v, w2_v, k_v, v_v, q_s, o_s,
               kv_sem, w_sem, w2_sem):
        def cp(src, dst, sem, r, pr, cc, pc):
            if not isinstance(r, int):
                r = pl.multiple_of(r, pr)
            return pltpu.make_async_copy(src.at[pl.ds(r, pr), pl.ds(cc, pc)],
                                         dst.at[pl.ds(r, pr), pl.ds(cc, pc)], sem)

        def wait_all(name, dst, sem):
            if scopes:
                with jax.named_scope("wait_" + name):
                    pltpu.make_async_copy(dst, dst, sem).wait()
            else:
                pltpu.make_async_copy(dst, dst, sem).wait()

        sched = kv_schedule(dk, dv, lag)

        def start_kv(j, s, half):
            n = len(sched) // 2
            for pair_ in sched[half * n:(half + 1) * n]:
                for prio, (w, g, pieces) in enumerate(pair_):
                    src, dst = ((k_hbm, k_v), (v_hbm, v_v))[w]
                    for r, nr in pieces:
                        pltpu.make_async_copy(src.at[4 * j + g, pl.ds(SK - W + r, nr), :],
                                              dst.at[s, g, pl.ds(r, nr)], kv_sem.at[w, s]).start(priority=prio)

        cx = pltpu.make_async_copy(x_hbm, x_v, w_sem.at[0]); cx.start()
        cc_ = pltpu.make_async_copy(c_hbm, c_v, w_sem.at[1]); cc_.start(priority=1)

        def p1(i, _):
            for half in range(2):
                for qd in range(4):
                    r = i * 8 + qd * 128
                    cp(wm_hbm, wm_v, w_sem.at[2], r, 8, half * 1536, 1536).start(priority=0)
                    cp(wq_hbm, wq_v, w_sem.at[3], r, 8, half * 2048, 2048).start(priority=1)
        lax.fori_loop(0, 16, p1, None)
        start_kv(0, 0, 0)
        cx.wait(); cc_.wait()
        wait_all("wm", wm_v, w_sem.at[2])
        wait_all("wq", wq_v, w_sem.at[3])
        x = x_v[...].astype(F32)
        if compute:
            c = c_v[...].astype(F32)
            sc = (c * jax.nn.sigmoid(c)).astype(BF)
            mod = _nn(sc, wm_v[...])
            sa, ca, ga, sb, cb, gb = [mod[:, i * D:(i + 1) * D] for i in range(6)]
            h = (_layernorm(x) * (1.0 + ca) + sa).astype(BF)
            q = _nn(h, wq_v[...])
            for hh in range(H):
                q_s[hh] = q[:, hh * DH:(hh + 1) * DH]
        start_kv(0, 0, 1)
        start_kv(1, 1, 0)

        def p2(i, _):
            for st in range(8):
                cp(wo_hbm, wo_v, w_sem.at[4], i * 32 + st * 512, 32, 0, D).start(priority=st % 2)
        scale = DH ** -0.5

        def head(bh, s, g):
            hh = lax.bitwise_and(bh, H - 1)
            qh = q_s[hh].astype(BF)
            sc_ = _nt(qh, k_v[s, g]) * scale
            m = jnp.max(sc_, axis=-1, keepdims=True)
            p = jnp.exp(sc_ - m)
            l = jnp.sum(p, axis=-1, keepdims=True)
            o_s[bh] = _nn(p.astype(BF), v_v[s, g]) / l

        def wchunk(name, ci):
            src, dst = {"w1": (w1_hbm, w1_v), "w3": (w3_hbm, w3_v), "w2": (w2_hbm, w2_v)}[name]
            if name == "w2":
                sem = w2_sem.at[ci // 4 if isinstance(ci, int) else lax.shift_right_logical(ci, 2)]
            else:
                sem = w_sem.at[5 if name == "w1" else 6]
            return cp(src, dst, sem, ci * 32, 32, 0, D)

        def tail_seg(n, n0, c0, n1, c1):
            if n == 1:
                if n0: wchunk(n0, c0).start(priority=0)
                if n1: wchunk(n1, c1).start(priority=1)
                return
            def body(i, _):
                if n0: wchunk(n0, c0 + i).start(priority=0)
                if n1: wchunk(n1, c1 + i).start(priority=1)
            lax.fori_loop(0, n, body, None)

        row = lax.broadcasted_iota(jnp.int32, (2, DH), 0)

        NQ = B * H // 4

        def quad(j, _):
            s = lax.bitwise_and(j, 1)
            wait_all("k", k_v.at[s], kv_sem.at[0, s])
            wait_all("v", v_v.at[s], kv_sem.at[1, s])
            if compute:
                head(4 * j, s, 0)
                head(4 * j + 1, s, 1)

            @pl.when(j < NQ - 1)
            def _():
                start_kv(j + 1, 1 - s, 1)

            @pl.when(j == NQ - 1)
            def _():
                for sg in segs[:nseg1]: tail_seg(*sg)

            if compute:
                head(4 * j + 2, s, 2)
                head(4 * j + 3, s, 3)

            @pl.when(j < NQ - 2)
            def _():
                start_kv(j + 2, s, 0)

            @pl.when(j == NQ - 2)
            def _():
                lax.fori_loop(0, 16, p2, None)

        lax.fori_loop(0, NQ, quad, None)
        for sg in segs[nseg1:]: tail_seg(*sg)
        wait_all("wo", wo_v, w_sem.at[4])
        if compute:
            o = jnp.concatenate([jnp.where(row == 0, o_s[hh], o_s[H + hh]) for hh in range(H)], axis=1).astype(BF)
            acc = _nn(o, wo_v[...])
        wait_all("w1", w1_v, w_sem.at[5])
        if compute:
            x1 = x + ga * acc
            h2 = (_layernorm(x1) * (1.0 + cb) + sb).astype(BF)
            g = _nt(h2, w1_v[...])
        wait_all("w3", w3_v, w_sem.at[6])
        if compute:
            u = _nt(h2, w3_v[...])
            a = (g * jax.nn.sigmoid(g) * u).astype(BF)
        y = jnp.zeros((2, D), F32)
        for grp in groups:
            for i in grp:
                n = min(128, F - i * 128)
                wait_all("w2_%d" % i, w2_v.at[pl.ds(i * 128, n)], w2_sem.at[i])
            if compute:
                for i in grp:
                    r0 = i * 128
                    n = min(128, F - r0)
                    y = y + _nn(a[:, r0:r0 + n], w2_v[pl.ds(r0, n), :])
        if compute:
            o_ref[...] = (x1 + gb * y).astype(o_ref.dtype)
        else:
            o_ref[...] = x.astype(o_ref.dtype)

    def f(A_x, A_k_cache, A_v_cache, A_wq, A_wo, B_x, B_w1, B_w3, B_w2, c, w_mod):
        a = [A_x.reshape(B, D), A_k_cache.reshape(B * H, SK, DH), A_v_cache.reshape(B * H, SK, DH),
             A_wq, A_wo, B_w1.T, B_w3.T, B_w2, c, w_mod]
        V = pltpu.VMEM
        out = pl.pallas_call(
            kernel, out_shape=jax.ShapeDtypeStruct((B, D), BF),
            in_specs=[pl.BlockSpec(memory_space=pltpu.HBM)] * len(a),
            scratch_shapes=[V((B, D), BF), V((B, D), BF), V((D, 6 * D), BF), V((D, H * DH), BF), V((H * DH, D), BF),
                            V((F, D), BF), V((F, D), BF), V((F, D), BF),
                            V((2, 4, W, DH), BF), V((2, 4, W, DH), BF), V((H, B, DH), F32), V((B * H, B, DH), F32),
                            pltpu.SemaphoreType.DMA((2, 2)), pltpu.SemaphoreType.DMA((8,)),
                            pltpu.SemaphoreType.DMA((11,))],
            compiler_params=pltpu.CompilerParams(vmem_limit_bytes=100 * 2**20, disable_bounds_checks=nobc),
        )(*a)
        return out.reshape(B, 1, D)
    return f


_impl = make(128,192,26)


@jax.jit
def pallas_adaLN_cond__sliding_block_cached__glu_gated_swiglu__decode_kernel(
    A_x, A_k_cache, A_v_cache, A_wq, A_wo, B_x, B_w1, B_w3, B_w2, c, w_mod,
):
    return _impl(A_x, A_k_cache, A_v_cache, A_wq, A_wo, B_x, B_w1, B_w3, B_w2, c, w_mod)
```

```python
import jax
import jax.numpy as jnp
from jax import lax
import jax.experimental.pallas as pl
import jax.experimental.pallas.tpu as pltpu

B, D, H, DH, SK, F = 2, 512, 32, 128, 16384, 1376
W = min(4096, max(256, SK // 4))
BF, F32 = jnp.bfloat16, jnp.float32

ROWS = 128
G = 4
NSTEP = B * H // G
NSLOT = 4
NS = 2 * G
SEG = 64
LAG = 26
K_SHIFT, V_SHIFT = 128, 192
FC = F // 32
NPIECE = pl.cdiv(F, 128)
Q0_FFN = (22, 25, 8)
Y_GROUPS = ((0, 1, 2, 3, 4), (5, 6, 7, 8), (9, 10))


def _layernorm(x, eps=1e-5):
    d = x - jnp.mean(x, axis=-1, keepdims=True)
    return d / jnp.sqrt(jnp.mean(d * d, axis=-1, keepdims=True) + eps)


def _silu(x):
    return x * jax.nn.sigmoid(x)


def _dot(a, b):
    return jnp.dot(a, b, preferred_element_type=F32)


def _dot_t(a, b):
    return lax.dot_general(a, b, (((1,), (1,)), ((), ())), preferred_element_type=F32)


def _interleave(lo, hi, n):
    m = pl.cdiv(hi - lo, n)
    return [lo + s * m + i for i in range(m) for s in range(n) if lo + s * m + i < hi]


def _head_index(j, g):
    return 2 * j + g % 2 + (g // 2) * H


def _kernel(x_hbm, k_hbm, v_hbm, wq_hbm, wo_hbm, w1_hbm, w3_hbm, w2_hbm, c_hbm, wm_hbm,
            out_ref,
            x_v, c_v, wm_v, wq_v, wo_v, w1_v, w3_v, w2_v, k_v, v_v, q_s, o_s,
            kv_sem, w_sem, w2_sem):
    x_sem, c_sem, wm_sem, wq_sem, wo_sem, w1_sem, w3_sem = (w_sem.at[i] for i in range(7))

    def tile_copy(src, dst, sem, r, nr, c, nc):
        idx = (pl.ds(r, nr), pl.ds(c, nc))
        return [pltpu.make_async_copy(src.at[idx], dst.at[idx], sem)]

    def kv_copy(j, stream, chunk):
        g, w = divmod(stream, 2)
        src, dst, shift = ((k_hbm, k_v, K_SHIFT), (v_hbm, v_v, V_SHIFT))[w]
        r = (chunk * ROWS - shift) & (W - 1)
        if not isinstance(chunk, int):
            pieces = ((pl.multiple_of(r, 64), ROWS),)
        elif r + ROWS <= W:
            pieces = ((r, ROWS),)
        else:
            pieces = ((r, W - r), (0, r + ROWS - W))
        s = j & (NSLOT - 1)
        return [pltpu.make_async_copy(src.at[_head_index(j, g), pl.ds(SK - W + r0, n), :],
                                      dst.at[s, g, pl.ds(r0, n)], kv_sem.at[w, s])
                for r0, n in pieces]

    def kv_half(j, upper):
        return lambda e: kv_copy(j, e % NS, 2 * (e // NS) + upper)

    def w_chunk(e, upper):
        return (2 * ((e % 8) * 8 + e // 8) + 1 + upper) % 128

    def wq_half(upper):
        def copy(e):
            row_tile, half = divmod(w_chunk(e, upper), 2)
            return tile_copy(wq_hbm, wq_v, wq_sem, row_tile * 8, 8, half * 2048, 2048)
        return copy

    def wo_half(upper):
        return lambda e: tile_copy(wo_hbm, wo_v, wo_sem, w_chunk(e, upper) * 32, 32, 0, D)

    def wm_copy(i):
        return tile_copy(wm_hbm, wm_v, wm_sem, (i // 2) * 8, 8, (i % 2) * 1536, 1536)

    def ffn_copy(m, i):
        src, dst = ((w1_hbm, w1_v), (w3_hbm, w3_v), (w2_hbm, w2_v))[m]
        return tile_copy(src, dst, (w1_sem, w3_sem, w2_sem.at[i // 4])[m], i * 32, 32, 0, D)

    ffn0 = [(m, i) for m in range(3) for i in range(Q0_FFN[m])]
    ffn1 = [(m, i) for m in range(3) for i in range(Q0_FFN[m], FC)]

    def start_pair(q0, q1):
        for cp in q0:
            cp.start(priority=0)
        for cp in q1:
            cp.start(priority=1)

    def wait_filled(buf, sem):
        pltpu.make_async_copy(buf, buf, sem).wait()

    def start_last_segment(lower, upper, next_upper, first):
        end = first + SEG
        for p in range(first, end):
            start_pair(lower(p), upper(p + LAG) if p + LAG < end else next_upper(p + LAG - end))

    def start_kv_first(j):
        def body(i, _):
            for st in range(NS):
                e = st + LAG
                start_pair(kv_copy(j, st, 2 * i), kv_copy(j, e % NS, 2 * (i + e // NS) + 1))
        lax.fori_loop(0, SEG // NS, body, None)

    def start_kv_second(j, next_upper):
        start_last_segment(kv_half(j, 0), kv_half(j, 1), next_upper, SEG)

    def start_ffn(lo, hi):
        for p in range(lo, hi):
            start_pair(ffn_copy(*ffn0[p]) if p < len(ffn0) else [],
                       ffn_copy(*ffn1[p + LAG]) if p + LAG < len(ffn1) else [])

    cx = pltpu.make_async_copy(x_hbm, x_v, x_sem)
    cc = pltpu.make_async_copy(c_hbm, c_v, c_sem)
    start_pair([cx], [cc])
    n0 = (128 + LAG) // 2
    wm0, wm1 = _interleave(0, n0, 3), _interleave(n0, 128, 2)
    assert len(wm0) - len(wm1) == LAG
    for p in range(n0):
        start_pair(wm_copy(wm0[p]), wm_copy(wm1[p]) if p < len(wm1) else wq_half(1)(p - len(wm1)))
    start_last_segment(wq_half(0), wq_half(1), kv_half(0, 1), 0)
    start_kv_first(0)
    cx.wait()
    cc.wait()
    wait_filled(wm_v, wm_sem)
    wait_filled(wq_v, wq_sem)

    x = x_v[...].astype(F32)
    mod = _dot(_silu(c_v[...].astype(F32)).astype(BF), wm_v[...])
    sa, ca, ga, sb, cb, gb = (mod[:, i * D:(i + 1) * D] for i in range(6))
    h = _layernorm(x) * (1.0 + ca) + sa
    q = _dot(h.astype(BF), wq_v[...])
    for hh in range(H):
        q_s[hh] = q[:, hh * DH:(hh + 1) * DH]

    start_kv_second(0, kv_half(1, 1))
    start_kv_first(1)

    def attend(j, g):
        s = j & (NSLOT - 1)
        qh = q_s[2 * j + g % 2].astype(BF)
        scores = _dot_t(qh, k_v[s, g]) * DH ** -0.5
        p = jnp.exp(scores - jnp.max(scores, axis=-1, keepdims=True))
        o_s[_head_index(j, g)] = _dot(p.astype(BF), v_v[s, g]) / jnp.sum(p, axis=-1, keepdims=True)

    def step(j, _):
        s = j & (NSLOT - 1)
        wait_filled(k_v.at[s], kv_sem.at[0, s])
        wait_filled(v_v.at[s], kv_sem.at[1, s])
        attend(j, 0)
        attend(j, 1)
        pl.when(j < NSTEP - 2)(lambda: start_kv_second(j + 1, kv_half(j + 2, 1)))
        pl.when(j == NSTEP - 2)(lambda: start_kv_second(NSTEP - 1, wo_half(1)))
        pl.when(j == NSTEP - 1)(lambda: start_ffn(0, SEG // 2))
        attend(j, 2)
        attend(j, 3)
        pl.when(j < NSTEP - 2)(lambda: start_kv_first(j + 2))
        pl.when(j == NSTEP - 2)(
            lambda: start_last_segment(wo_half(0), wo_half(1), lambda e: ffn_copy(*ffn1[e]), 0))
        pl.when(j == NSTEP - 1)(lambda: start_ffn(SEG // 2, max(len(ffn0), len(ffn1) - LAG)))

    lax.fori_loop(0, NSTEP, step, None)

    wait_filled(wo_v, wo_sem)
    row = lax.broadcasted_iota(jnp.int32, (B, DH), 0)
    o = jnp.concatenate([jnp.where(row == 0, o_s[hh], o_s[H + hh]) for hh in range(H)], axis=1)
    x = x + ga * _dot(o.astype(BF), wo_v[...])
    h = (_layernorm(x) * (1.0 + cb) + sb).astype(BF)
    wait_filled(w1_v, w1_sem)
    gate = _dot_t(h, w1_v[...])
    wait_filled(w3_v, w3_sem)
    a = (_silu(gate) * _dot_t(h, w3_v[...])).astype(BF)
    y = jnp.zeros((B, D), F32)
    for group in Y_GROUPS:
        spans = [(i * 128, min(128, F - i * 128)) for i in group]
        for i, (r, n) in zip(group, spans):
            wait_filled(w2_v.at[pl.ds(r, n)], w2_sem.at[i])
        for r, n in spans:
            y = y + _dot(a[:, r:r + n], w2_v[pl.ds(r, n), :])
    out_ref[...] = (x + gb * y).astype(out_ref.dtype)


@jax.jit
def pallas_adaLN_cond__sliding_block_cached__glu_gated_swiglu__decode_kernel(
    A_x: jax.Array,
    A_k_cache: jax.Array,
    A_v_cache: jax.Array,
    A_wq: jax.Array,
    A_wo: jax.Array,
    B_x: jax.Array,
    B_w1: jax.Array,
    B_w3: jax.Array,
    B_w2: jax.Array,
    c: jax.Array,
    w_mod: jax.Array,
):
    del B_x
    args = (A_x.reshape(B, D), A_k_cache.reshape(B * H, SK, DH), A_v_cache.reshape(B * H, SK, DH),
            A_wq, A_wo, B_w1.T, B_w3.T, B_w2, c, w_mod)
    vmem = pltpu.VMEM
    out = pl.pallas_call(
        _kernel,
        out_shape=jax.ShapeDtypeStruct((B, D), A_x.dtype),
        in_specs=[pl.BlockSpec(memory_space=pltpu.HBM)] * len(args),
        scratch_shapes=[
            vmem((B, D), BF), vmem((B, D), BF),
            vmem((D, 6 * D), BF), vmem((D, H * DH), BF), vmem((H * DH, D), BF),
            vmem((F, D), BF), vmem((F, D), BF), vmem((F, D), BF),
            vmem((NSLOT, G, W, DH), BF), vmem((NSLOT, G, W, DH), BF),
            vmem((H, B, DH), F32), vmem((B * H, B, DH), F32),
            pltpu.SemaphoreType.DMA((2, NSLOT)),
            pltpu.SemaphoreType.DMA((7,)),
            pltpu.SemaphoreType.DMA((NPIECE,)),
        ],
        compiler_params=pltpu.CompilerParams(vmem_limit_bytes=64 * 2**20),
    )(*args)
    return out.reshape(B, 1, D)
```
